```python
import os as _os
_os.environ.setdefault("JAX_PLATFORMS", "cpu")
import jax
import jax.numpy as jnp

def _softmax(x, axis=-1):
    return jax.nn.softmax(x, axis=axis)
def _gelu(x):
    return jax.nn.gelu(x, approximate=True)
def _silu(x):
    return jax.nn.silu(x)
def _sigmoid(x):
    return jax.nn.sigmoid(x)
def _layernorm(x, axis=-1, eps=1e-5):
    m = jnp.mean(x, axis=axis, keepdims=True)
    v = jnp.var(x, axis=axis, keepdims=True)
    return (x - m) / jnp.sqrt(v + eps)
def _scatter_add(tgt, idx, src, axis=0):
    return tgt.at[idx].add(src)
def _segment_sum(src, seg, n):
    return jax.ops.segment_sum(src, seg, n)
class _Rng:
    def __init__(self, key):
        self._k = key
    def _next(self):
        self._k, sub = jax.random.split(self._k)
        return sub
    def normal(self, shape):
        return jax.random.normal(self._next(), shape, dtype=jnp.bfloat16)
    def randint(self, lo, hi, shape):
        return jax.random.randint(self._next(), shape, lo, hi, dtype=jnp.int32)
    def uniform(self, shape, lo=0.0, hi=1.0):
        return jax.random.uniform(self._next(), shape, jnp.bfloat16, lo, hi)
    def permutation(self, n):
        return jax.random.permutation(self._next(), n)


kernel_name = 'concat_heads__gqa_block_cached__mha_block_cached__near_ridge'

def setup_inputs():
    _rng = _Rng(jax.random.key(int.from_bytes(__import__("os").urandom(4), "little")))
    _w = (lambda a: (lambda t: t.astype(jnp.bfloat16) if jnp.issubdtype(t.dtype, jnp.floating) else t)(jnp.asarray(a)))
    def _A_setup():
        B, Sq, D = 8, 48, 512
        Hq, Hkv, Sk, Dh = 32, 8, 1024, 128
        assert Hq % Hkv == 0, (Hq, Hkv)
        return {
            "x": _w((lambda *s: _rng.normal(s) * 0.8)(B, Sq, D)),
            "k_cache": _w((lambda *s: _rng.normal(s) * 0.8)(B, Hkv, Sk, Dh)),
            "v_cache": _w((lambda *s: _rng.normal(s) * 0.05)(B, Hkv, Sk, Dh)),
            "wq": _w((lambda *s: _rng.normal(s) * 0.8)(D, Hq * Dh) * (D ** -0.5)),
            "wo": _w((lambda *s: _rng.normal(s) * 0.05)(Hq * Dh, D) * ((Hq * Dh) ** -0.5)),
        }
    _A_in = _A_setup()

    def _B_setup():
        B, Sq, D = 8, 48, 512
        H, Sk, Dh = 32, 1024, 128
        return {
            "x": _w((lambda *s: _rng.normal(s) * 0.8)(B, Sq, D)),
            "k_cache": _w((lambda *s: _rng.normal(s) * 0.8)(B, H, Sk, Dh)),
            "v_cache": _w((lambda *s: _rng.normal(s) * 0.05)(B, H, Sk, Dh)),
            "wq": _w((lambda *s: _rng.normal(s) * 0.8)(D, H * Dh) * (D ** -0.5)),
            "wo": _w((lambda *s: _rng.normal(s) * 0.05)(H * Dh, D) * ((H * Dh) ** -0.5)),
        }
    _B_in = _B_setup()

    return {
        "A_x": _A_in["x"],
        "A_k_cache": _A_in["k_cache"],
        "A_v_cache": _A_in["v_cache"],
        "A_wq": _A_in["wq"],
        "A_wo": _A_in["wo"],
        "B_x": _B_in["x"],
        "B_k_cache": _B_in["k_cache"],
        "B_v_cache": _B_in["v_cache"],
        "B_wq": _B_in["wq"],
        "B_wo": _B_in["wo"],
    }

def reference(A_x, A_k_cache, A_v_cache, A_wq, A_wo, B_x, B_k_cache, B_v_cache, B_wq, B_wo):
    def _A_ref(x, k_cache, v_cache, wq, wo):
        B, Sq, D = x.shape
        Hq, Dh = 32, 128
        Hkv = k_cache.shape[1]
        rep = Hq // Hkv
        q = (lambda x, *d: x.transpose(*d))((x @ wq).reshape(B, Sq, Hq, Dh), 0, 2, 1, 3)
        k = jnp.repeat(k_cache, rep, axis=1)
        v = jnp.repeat(v_cache, rep, axis=1)
        scores = jnp.einsum("bhqd,bhkd->bhqk", q, k) * (Dh ** -0.5)
        p = _softmax(scores, axis=-1)
        o = jnp.einsum("bhqk,bhkd->bhqd", p, v)
        return (lambda x, *d: x.transpose(*d))(o, 0, 2, 1, 3).reshape(B, Sq, Hq * Dh) @ wo

    def _B_ref(x, k_cache, v_cache, wq, wo):
        B, Sq, D = x.shape
        H, Dh = 32, 128
        q = (lambda x, *d: x.transpose(*d))((x @ wq).reshape(B, Sq, H, Dh), 0, 2, 1, 3)
        scores = jnp.einsum("bhqd,bhkd->bhqk", q, k_cache) * (Dh ** -0.5)
        p = _softmax(scores, axis=-1)
        o = jnp.einsum("bhqk,bhkd->bhqd", p, v_cache)
        return (lambda x, *d: x.transpose(*d))(o, 0, 2, 1, 3).reshape(B, Sq, H * Dh) @ wo

    a = _A_ref(A_x, A_k_cache, A_v_cache, A_wq, A_wo)
    b = _B_ref(B_x, B_k_cache, B_v_cache, B_wq, B_wo)
    return jnp.concatenate([a, b], axis=-1)
```

```python
import functools
import math

import jax
import jax.numpy as jnp
from jax import lax
from jax.experimental import pallas as pl
from jax.experimental.pallas import tpu as pltpu

NB, SQ, D = 8, 48, 512
HQ, HKV, SK, DH = 32, 8, 1024, 128
REP = HQ // HKV
GW = REP * DH
NSTEP = HKV * NB
CH = 128
WCH = 32
QSCALE = float(DH ** -0.5 * math.log2(math.e))


def _attend(q, k, v):
    s = lax.dot_general(q, k, (((1,), (1,)), ((), ())), preferred_element_type=jnp.float32)
    m = jnp.max(s, axis=-1, keepdims=True)
    p = jnp.exp2(s - m)
    l = jnp.sum(p, axis=-1, keepdims=True)
    o = jnp.dot(p.astype(jnp.bfloat16), v, preferred_element_type=jnp.float32)
    return (o * (1.0 / l)).astype(jnp.bfloat16)


def kv_order(name):
    nr = SK // CH
    if name == "r_slab_a":
        sl = [0, 4, 2, 6, 8, 9, 1, 5, 3, 7]
        return [(s, r) for r in range(nr) for s in sl]
    if name == "r_slab_b":
        sl = [0, 2, 4, 6, 8, 9, 1, 3, 5, 7]
        return [(s, r) for r in range(nr) for s in sl]
    if name == "r_slab_c":
        sl = [0, 6, 8, 2, 4, 1, 7, 9, 3, 5]
        return [(s, r) for r in range(nr) for s in sl]
    if name == "plain":
        return [(s, r) for r in range(nr) for s in range(10)]
    raise ValueError(name)


def make(nslot=4, lag=2, nburst=3, order="r_slab_a", compute=True, prio=True, nbc=True, flags=None):
    def kernel(xa, ka, va, wqa, woa, xb, kb, vb, wqb, wob, out,
               xbuf, wbuf, kvbuf, acc, obuf, sem_x, sem_w, sem_kv, sem_o):

        def kv_copies(s, slot):
            g = s // NB
            b = s % NB
            cps = []
            for slab, r in kv_order(order):
                rows = pl.ds(r * CH, CH)
                if slab < 4:
                    src = kb.at[b, g * REP + slab, rows]
                elif slab < 8:
                    src = vb.at[b, g * REP + (slab - 4), rows]
                elif slab == 8:
                    src = ka.at[b, g, rows]
                else:
                    src = va.at[b, g, rows]
                cps.append(pltpu.make_async_copy(src, kvbuf.at[slot, slab, rows], sem_kv.at[slot]))
            return cps

        def w_copies(g, c0, nc):
            cps = []
            col = pl.ds(pl.multiple_of(g * GW, GW), GW)
            for i in range(nc):
                r0 = (c0 + i) * WCH
                if not isinstance(r0, int):
                    r0 = pl.multiple_of(r0, WCH)
                rows = pl.ds(r0, WCH)
                orow = g * GW + r0
                if not isinstance(orow, int):
                    orow = pl.multiple_of(orow, WCH)
                orows = pl.ds(orow, WCH)
                sem = sem_w.at[g % 2]
                cps.append(pltpu.make_async_copy(wqa.at[rows, col], wbuf.at[g, 0, rows], sem))
                cps.append(pltpu.make_async_copy(wqb.at[rows, col], wbuf.at[g, 1, rows], sem))
                cps.append(pltpu.make_async_copy(woa.at[orows], wbuf.at[g, 2, rows], sem))
                cps.append(pltpu.make_async_copy(wob.at[orows], wbuf.at[g, 3, rows], sem))
            return cps

        def start_all(cps, first=0):
            for i, c in enumerate(cps):
                c.start(priority=((i + first) % 2) if prio else 0)

        pro = []
        for i in range(NB * SQ // WCH):
            rows = pl.ds(i * WCH, WCH)
            pro.append(pltpu.make_async_copy(xa.at[rows], xbuf.at[0, rows], sem_x))
            pro.append(pltpu.make_async_copy(xb.at[rows], xbuf.at[1, rows], sem_x))
        start_all(pro)
        start_all(w_copies(0, 0, 16))

        def pro_body(s, c):
            start_all(kv_copies(s, s))

            @pl.when(s >= 1)
            def _():
                start_all(w_copies(1, (s - 1) * 2, 2))
            return c
        lax.fori_loop(0, lag, pro_body, 0)

        acc[...] = jnp.zeros(acc.shape, acc.dtype)
        pltpu.make_async_copy(xbuf, xbuf, sem_x).wait()

        def step(t, carry):
            g = t // NB
            b = t % NB
            slot = t % nslot
            s = t + lag
            sslot = s % nslot

            @pl.when(b == 0)
            def _():
                pltpu.make_async_copy(wbuf.at[g], wbuf.at[g], sem_w.at[g % 2]).wait()

            pltpu.make_async_copy(kvbuf.at[slot], kvbuf.at[slot], sem_kv.at[slot]).wait()

            def burst(i):
                @pl.when(s < NSTEP)
                def _():
                    cps = kv_copies(s, sslot)
                    n = len(cps)
                    lo = (n * i // nburst) // 2 * 2
                    hi = (n * (i + 1) // nburst) // 2 * 2
                    start_all(cps[lo:hi])

                if i == nburst - 1:
                    @pl.when(s <= NSTEP - NB)
                    def _():
                        u = s + NB - 1
                        start_all(w_copies(u // NB, (u % NB) * 2, 2))

            rows = pl.ds(pl.multiple_of(b * SQ, SQ), SQ)
            pieces = {}

            def piece_a():
                q = jnp.dot(xbuf[0, rows, :], wbuf[g, 0], preferred_element_type=jnp.float32)
                q = (q * QSCALE).astype(jnp.bfloat16)
                q = jnp.concatenate([q[:, j * DH:(j + 1) * DH] for j in range(REP)], axis=0)
                o = _attend(q, kvbuf[slot, 8], kvbuf[slot, 9])
                o = jnp.concatenate([o[j * SQ:(j + 1) * SQ] for j in range(REP)], axis=1)
                acc[0, rows, :] += jnp.dot(o, wbuf[g, 2], preferred_element_type=jnp.float32)

            def piece_b():
                q = jnp.dot(xbuf[1, rows, :], wbuf[g, 1], preferred_element_type=jnp.float32)
                q = (q * QSCALE).astype(jnp.bfloat16)
                o = [_attend(q[:, j * DH:(j + 1) * DH], kvbuf[slot, j], kvbuf[slot, 4 + j]) for j in range(REP)]
                o = jnp.concatenate(o, axis=1)
                acc[1, rows, :] += jnp.dot(o, wbuf[g, 3], preferred_element_type=jnp.float32)

            if nburst == 1:
                burst(0)
                if compute:
                    piece_a()
                    piece_b()
            elif nburst == 2:
                burst(0)
                if compute:
                    piece_a()
                burst(1)
                if compute:
                    piece_b()
            elif nburst == 3:
                burst(0)
                if compute:
                    piece_a()
                burst(1)
                if compute:
                    q = jnp.dot(xbuf[1, rows, :], wbuf[g, 1], preferred_element_type=jnp.float32)
                    q = (q * QSCALE).astype(jnp.bfloat16)
                    o = [_attend(q[:, j * DH:(j + 1) * DH], kvbuf[slot, j], kvbuf[slot, 4 + j]) for j in range(2)]
                burst(2)
                if compute:
                    o += [_attend(q[:, j * DH:(j + 1) * DH], kvbuf[slot, j], kvbuf[slot, 4 + j]) for j in range(2, 4)]
                    o = jnp.concatenate(o, axis=1)
                    acc[1, rows, :] += jnp.dot(o, wbuf[g, 3], preferred_element_type=jnp.float32)

            @pl.when(g == HKV - 1)
            def _():
                obuf[rows, 0:D] = acc[0, rows, :].astype(jnp.bfloat16)
                obuf[rows, D:2 * D] = acc[1, rows, :].astype(jnp.bfloat16)
                pltpu.make_async_copy(obuf.at[rows], out.at[rows], sem_o).start()
            return carry

        lax.fori_loop(0, NSTEP, step, 0)
        pltpu.make_async_copy(obuf, out, sem_o).wait()

    def f(A_x, A_k, A_v, A_wq, A_wo, B_x, B_k, B_v, B_wq, B_wo):
        hbm = pl.BlockSpec(memory_space=pltpu.HBM)
        o = pl.pallas_call(
            kernel,
            out_shape=jax.ShapeDtypeStruct((NB * SQ, 2 * D), jnp.bfloat16),
            in_specs=[hbm] * 10,
            out_specs=hbm,
            scratch_shapes=[
                pltpu.VMEM((2, NB * SQ, D), jnp.bfloat16),
                pltpu.VMEM((HKV, 4, GW, GW), jnp.bfloat16),
                pltpu.VMEM((nslot, 10, SK, DH), jnp.bfloat16),
                pltpu.VMEM((2, NB * SQ, D), jnp.float32),
                pltpu.VMEM((NB * SQ, 2 * D), jnp.bfloat16),
                pltpu.SemaphoreType.DMA,
                pltpu.SemaphoreType.DMA((2,)),
                pltpu.SemaphoreType.DMA((nslot,)),
                pltpu.SemaphoreType.DMA,
            ],
            compiler_params=pltpu.CompilerParams(
                vmem_limit_bytes=100 * 1024 * 1024, disable_bounds_checks=nbc, flags=flags),
        )(A_x.reshape(NB * SQ, D), A_k, A_v, A_wq, A_wo, B_x.reshape(NB * SQ, D), B_k, B_v, B_wq, B_wo)
        return o.reshape(NB, SQ, 2 * D)

    return f


_impl = make(nburst=3, order="r_slab_c")


@jax.jit
def pallas_concat_heads__gqa_block_cached__mha_block_cached__near_ridge_kernel(
    A_x, A_k_cache, A_v_cache, A_wq, A_wo, B_x, B_k_cache, B_v_cache, B_wq, B_wo,
):
    return _impl(A_x, A_k_cache, A_v_cache, A_wq, A_wo, B_x, B_k_cache, B_v_cache, B_wq, B_wo)
```

```python
import contextlib
import math

import jax
import jax.numpy as jnp
from jax import lax
from jax.experimental import pallas as pl
from jax.experimental.pallas import tpu as pltpu

NB, SQ, D = 8, 48, 512
HQ, HKV, SK, DH = 32, 8, 1024, 128
REP = HQ // HKV
GW = REP * DH
NSTEP = 64
CH = 128
NCH = SK // CH
QSCALE = float(DH ** -0.5 * math.log2(math.e))
BF16, F32 = jnp.bfloat16, jnp.float32


def _qk(q, k):
    return lax.dot_general(q, k, (((1,), (1,)), ((), ())), preferred_element_type=F32)


def _softmax(s):
    m = jnp.max(s, axis=-1, keepdims=True)
    p = jnp.exp2(s - m)
    l = jnp.sum(p, axis=-1, keepdims=True)
    return p.astype(BF16), 1.0 / l


def _pv(pr, v):
    return (jnp.dot(pr[0], v, preferred_element_type=F32) * pr[1]).astype(BF16)


def _ds(start, size, align):
    if isinstance(start, int):
        return pl.ds(start, size)
    return pl.ds(pl.multiple_of(start, align), size)


def make(nslot=4, offc=2, a_first=11, compute=True, dma=True, nbc=True, nsc=True, flags=None,
         endgame="simple", out_split="par", bursts=(32, 32), scopes=False, asplit=2, a_pos="end",
         x_prio=(1, 1), korder=None, zero="pro", xrows=48, wpat=(4, 32)):
    lag = 2
    if scopes is True:
        scope = jax.named_scope
    elif scopes:
        scope = lambda n: jax.named_scope(n) if n in scopes else contextlib.nullcontext()
    else:
        scope = lambda n: contextlib.nullcontext()

    def kernel(xa, ka, va, wqa, woa, xb, kb, vb, wqb, wob, out,
               xbuf, wqbuf, wobuf, abuf, bbuf, acc, obuf, sem_x, sem_wq, sem_wo, sem_a, sem_bk, sem_bv, sem_o):

        def start(src, dst, sem, prio):
            if dma:
                pltpu.make_async_copy(src, dst, sem).start(priority=prio)

        def wait(buf, sem):
            if dma:
                pltpu.make_async_copy(buf, buf, sem).wait()

        def issue_b(s, lo, hi, unit_major=False):
            h = s // 2
            par = s % 2
            slot = s % nslot
            for n in range(lo, hi):
                arr = n % 2
                m = n // 2
                r, i = m // 4, m % 4
                if korder is not None:
                    i = korder[arr][i]
                if unit_major and arr == 1:
                    i, r = m // NCH, m % NCH
                rows = pl.ds(r * CH, CH)
                sem = sem_bk.at[slot] if arr == 0 else sem_bv.at[slot * 4 + i]
                start((kb, vb)[arr].at[2 * i + par, h, rows], bbuf.at[slot, arr, i, rows], sem, arr)

        def issue_a(a):
            g = a // NCH
            rows = _ds((a % NCH) * CH, CH, CH)
            for b in range(NB):
                for arr in range(2):
                    start((ka, va)[arr].at[b, g, rows], abuf.at[g, arr, b, rows], sem_a.at[g], arr)

        xn = SQ // xrows
        for b in range(NB):
            for c in range(xn):
                rows = pl.ds(b * SQ + c * xrows, xrows)
                start(xa.at[rows], xbuf.at[0, rows], sem_x, x_prio[0])
                start(xb.at[rows], xbuf.at[1, pl.ds(((b % 2) * 4 + b // 2) * SQ + c * xrows, xrows)], sem_x, x_prio[1])

        def w_chunk(i, n):
            ns, step = wpat
            grp = 128 // (ns * step)
            return (i // step) * (ns * step) + n * step + i % step

        def wq_body(i, c):
            for n in range(wpat[0]):
                ch = w_chunk(i, n)
                rows = _ds((ch // 2) * 8, 8, 8)
                cols = _ds((ch % 2) * 2048, 2048, 2048)
                for w in range(2):
                    start((wqa, wqb)[w].at[rows, cols], wqbuf.at[w, rows, cols], sem_wq, w)
            return c

        def wo_body(i, c):
            for n in range(wpat[0]):
                rows = _ds(w_chunk(i, n) * 32, 32, 32)
                for w in range(2):
                    start((woa, wob)[w].at[rows], wobuf.at[w, rows], sem_wo, w)
            return c
        with scope("wloop"):
            lax.fori_loop(0, 128 // wpat[0], wq_body, 0)
            lax.fori_loop(0, 128 // wpat[0], wo_body, 0)

        def a_body(a, c):
            issue_a(a)
            return c
        with scope("aloop"):
            lax.fori_loop(0, a_first, a_body, 0)

        if offc < lag:
            def b_body(s, c):
                issue_b(s, 0, 64)
                return c
            lax.fori_loop(0, lag - offc, b_body, 0)

        with scope("zero"):
            def z_body(i, c):
                rows = _ds(i * SQ, SQ, SQ)
                acc[0, rows, :] = jnp.zeros((SQ, D), F32)
                acc[1, rows, :] = jnp.zeros((SQ, D), F32)
                return c
            lax.fori_loop(0, NB, z_body, 0)
        with scope("waitW"):
            wait(xbuf, sem_x)
            wait(wqbuf, sem_wq)
            wait(wobuf, sem_wo)

        def piece_a(u):
            g = u // NB
            b = u % NB

            @pl.when(b == 0)
            def _():
                wait(abuf.at[g], sem_a.at[g])

            if not compute:
                return
            rows = _ds(b * SQ, SQ, SQ)
            grp = _ds(g * GW, GW, GW)
            q = jnp.dot(xbuf[0, rows, :], wqbuf[0, :, grp], preferred_element_type=F32)
            q = (q * QSCALE).astype(BF16)
            n = REP // asplit
            qs = [jnp.concatenate([q[:, j * DH:(j + 1) * DH] for j in range(c * n, (c + 1) * n)], axis=0)
                  for c in range(asplit)]
            pr = [_softmax(_qk(qc, abuf[g, 0, b])) for qc in qs]
            o = [_pv(p, abuf[g, 1, b]) for p in pr]
            o = jnp.concatenate([oc[j * SQ:(j + 1) * SQ] for oc in o for j in range(n)], axis=1)
            acc[0, rows, :] += jnp.dot(o, wobuf[0, grp, :], preferred_element_type=F32)

        def b_q(t):
            rows = _ds((t % 2) * 4 * SQ, 4 * SQ, 4 * SQ)
            head = _ds((t // 2) * DH, DH, DH)
            q = jnp.dot(xbuf[1, rows, :], wqbuf[1, :, head], preferred_element_type=F32)
            return (q * QSCALE).astype(BF16)

        def b_out(t, o):
            rows = _ds((t % 2) * 4 * SQ, 4 * SQ, 4 * SQ)
            head = _ds((t // 2) * DH, DH, DH)
            return rows, jnp.dot(jnp.concatenate(o, axis=0), wobuf[1, head, :], preferred_element_type=F32)

        def finish_a():
            def body(i, c):
                rows = _ds(i * SQ, SQ, SQ)
                obuf[rows, 0:D] = acc[0, rows, :].astype(BF16)
                return c
            lax.fori_loop(0, NB, body, 0)

        def finish_b(par, val):
            for i in range(4):
                obuf[pl.ds((2 * i + par) * SQ, SQ), D:2 * D] = val[i * SQ:(i + 1) * SQ].astype(BF16)

        def write(rows, cols):
            pltpu.make_async_copy(obuf.at[rows, cols], out.at[rows, cols], sem_o).start()

        def write_early():
            if out_split == "par":
                for i in range(4):
                    write(pl.ds(2 * i * SQ, SQ), slice(None))
            elif out_split == "a_par":
                write(slice(None), pl.ds(0, D))
                for i in range(4):
                    write(pl.ds(2 * i * SQ, SQ), pl.ds(D, D))
            elif out_split == "par_a":
                for i in range(4):
                    write(pl.ds(2 * i * SQ, SQ), slice(None))
                for i in range(4):
                    write(pl.ds((2 * i + 1) * SQ, SQ), pl.ds(0, D))

        def write_late():
            if out_split == "par":
                for i in range(4):
                    write(pl.ds((2 * i + 1) * SQ, SQ), slice(None))
            elif out_split in ("a_par", "par_a"):
                for i in range(4):
                    write(pl.ds((2 * i + 1) * SQ, SQ), pl.ds(D, D))
            else:
                pltpu.make_async_copy(obuf, out, sem_o).start()

        last_plain = NSTEP if endgame.startswith("simple") else NSTEP - 1

        def step(u, carry):
            def burst(lo, hi):
                cond = u < last_plain - lag + offc
                if offc > lag:
                    cond = jnp.logical_and(u >= offc - lag, cond)

                @pl.when(cond)
                def _():
                    issue_b(u + lag - offc, lo, hi)
                if last_plain < NSTEP:
                    @pl.when(u == NSTEP - 1 - lag + offc)
                    def _():
                        issue_b(NSTEP - 1, lo, hi, unit_major=True)

            def burst_a():
                with scope("burstA"):
                    @pl.when(u + a_first < NSTEP)
                    def _():
                        issue_a(u + a_first)

            if a_pos == "start":
                burst_a()
            with scope("burst0"):
                burst(0, bursts[0])

            with scope("pieceA"):
                @pl.when(u < NSTEP)
                def _():
                    piece_a(u)

            if a_pos == "mid":
                burst_a()
            with scope("burst1"):
                burst(bursts[0], 64)

            if endgame == "simple2":
                @pl.when(u == NSTEP)
                def _():
                    finish_a()

            def piece_b():
                t = u - offc
                slot = t % nslot
                with scope("waitB"):
                    wait(bbuf.at[slot, 0], sem_bk.at[slot])
                    for i in range(4):
                        wait(bbuf.at[slot, 1, i], sem_bv.at[slot * 4 + i])
                if endgame == "simple2":
                    @pl.when(t == NSTEP - 1)
                    def _():
                        finish_b(0, acc[1, 0:4 * SQ, :])
                        write_early()
                with scope("pieceB"):
                    if compute:
                        q = b_q(t)
                        pr = [_softmax(_qk(q[i * SQ:(i + 1) * SQ], bbuf[slot, 0, i])) for i in range(4)]
                        o = [_pv(pr[i], bbuf[slot, 1, i]) for i in range(4)]
                        rows, val = b_out(t, o)
                        acc[1, rows, :] += val

            if offc > 0:
                pl.when(u >= offc)(piece_b)
            else:
                piece_b()

            if a_pos == "end":
                burst_a()
            return carry

        if endgame == "simple":
            with scope("main"):
                lax.fori_loop(0, NSTEP + offc, step, 0)
            with scope("finish"):
                finish_a()
                finish_b(0, acc[1, 0:4 * SQ, :])
                finish_b(1, acc[1, 4 * SQ:8 * SQ, :])
                pltpu.make_async_copy(obuf, out, sem_o).start()
        elif endgame == "simple2":
            with scope("main"):
                lax.fori_loop(0, NSTEP + offc, step, 0)
            with scope("finish"):
                finish_b(1, acc[1, 4 * SQ:8 * SQ, :])
                write_late()
        else:
            lax.fori_loop(0, NSTEP - 1 + offc, step, 0)
            t = NSTEP - 1
            slot = t % nslot
            with scope("fin0"):
                finish_a()
                finish_b(0, acc[1, 0:4 * SQ, :])
                q = b_q(t)
            with scope("waitK"):
                wait(bbuf.at[slot, 0], sem_bk.at[slot])
            with scope("scores"):
                pr = [_softmax(_qk(q[i * SQ:(i + 1) * SQ], bbuf[slot, 0, i])) for i in range(4)]
            o = []
            ew = int(endgame[-1])
            for i in range(4):
                with scope(f"waitV{i}"):
                    wait(bbuf.at[slot, 1, i], sem_bv.at[slot * 4 + i])
                if i == ew:
                    write_early()
                with scope(f"pv{i}"):
                    o.append(_pv(pr[i], bbuf[slot, 1, i]))
            with scope("fin1"):
                _, val = b_out(t, o)
                finish_b(1, acc[1, 4 * SQ:8 * SQ, :] + val)
                write_late()
        with scope("waitO"):
            pltpu.make_async_copy(obuf, out, sem_o).wait()

    def f(A_x, A_k, A_v, A_wq, A_wo, B_x, B_k, B_v, B_wq, B_wo):
        hbm = pl.BlockSpec(memory_space=pltpu.HBM)
        o = pl.pallas_call(
            kernel,
            out_shape=jax.ShapeDtypeStruct((NB * SQ, 2 * D), BF16),
            in_specs=[hbm] * 10,
            out_specs=hbm,
            scratch_shapes=[
                pltpu.VMEM((2, NB * SQ, D), BF16),
                pltpu.VMEM((2, D, HQ * DH), BF16),
                pltpu.VMEM((2, HQ * DH, D), BF16),
                pltpu.VMEM((HKV, 2, NB, SK, DH), BF16),
                pltpu.VMEM((nslot, 2, 4, SK, DH), BF16),
                pltpu.VMEM((2, NB * SQ, D), F32),
                pltpu.VMEM((NB * SQ, 2 * D), BF16),
                pltpu.SemaphoreType.DMA,
                pltpu.SemaphoreType.DMA,
                pltpu.SemaphoreType.DMA,
                pltpu.SemaphoreType.DMA((HKV,)),
                pltpu.SemaphoreType.DMA((nslot,)),
                pltpu.SemaphoreType.DMA((nslot * 4,)),
                pltpu.SemaphoreType.DMA,
            ],
            compiler_params=pltpu.CompilerParams(
                vmem_limit_bytes=100 * 1024 * 1024, disable_bounds_checks=nbc,
                disable_semaphore_checks=nsc, flags=flags),
        )(A_x.reshape(NB * SQ, D), A_k, A_v, A_wq, A_wo, B_x.reshape(NB * SQ, D), B_k, B_v, B_wq, B_wo)
        return o.reshape(NB, SQ, 2 * D)

    return f


_impl = make(endgame="simple2", out_split="a_par", xrows=24, korder=((0, 1, 2, 3), (3, 0, 1, 2)))


@jax.jit
def pallas_concat_heads__gqa_block_cached__mha_block_cached__near_ridge_kernel(
    A_x, A_k_cache, A_v_cache, A_wq, A_wo, B_x, B_k_cache, B_v_cache, B_wq, B_wo,
):
    return _impl(A_x, A_k_cache, A_v_cache, A_wq, A_wo, B_x, B_k_cache, B_v_cache, B_wq, B_wo)
```

```python
import math

import jax
import jax.numpy as jnp
from jax import lax
import jax.experimental.pallas as pl
import jax.experimental.pallas.tpu as pltpu

NB, SQ, D = 8, 48, 512
HQ, HKV, SK, DH = 32, 8, 1024, 128
REP = HQ // HKV
GW = REP * DH
NSTEP = HKV * NB
HB = NB // 2

CH = 128
NCH = SK // CH
WO_ROWS = 32
WQ_ROWS, WQ_COLS = 8, 2048
W_CHUNKS = HQ * DH // WO_ROWS
W_STREAMS = 4

LAG = 2
NSLOT = 4
A_AHEAD = 11
V_SPLIT = 6 * CH
B_BASE = HKV * 2 * NB

Q_SCALE = DH ** -0.5 * math.log2(math.e)

BF16, F32 = jnp.bfloat16, jnp.float32


def _rows(index, size):
    if isinstance(index, int):
        return pl.ds(index * size, size)
    return pl.ds(pl.multiple_of(index * size, size), size)


def _softmax_scores(q, k):
    s = lax.dot_general(q, k, (((1,), (1,)), ((), ())), preferred_element_type=F32)
    p = jnp.exp2(s - jnp.max(s, axis=-1, keepdims=True))
    return p.astype(BF16), 1.0 / jnp.sum(p, axis=-1, keepdims=True)


def _weighted_values(scores, v):
    p, inv_sum = scores
    return (jnp.dot(p, v, preferred_element_type=F32) * inv_sum).astype(BF16)


def _kernel(xa_hbm, ka_hbm, va_hbm, wqa_hbm, woa_hbm,
            xb_hbm, kb_hbm, vb_hbm, wqb_hbm, wob_hbm, out_hbm,
            x_buf, wq_buf, wo_buf, kv_buf, acc, out_buf,
            sem_x, sem_wq, sem_wo, sem_a, sem_k, sem_v, sem_out):

    def fetch(src, dst, sem, priority):
        pltpu.make_async_copy(src, dst, sem).start(priority=priority)

    def wait_filled(buf, sem):
        pltpu.make_async_copy(buf, buf, sem).wait()

    def fetch_a(a, which, b, priority):
        g = a // NCH
        rows = _rows(a % NCH, CH)
        fetch((ka_hbm, va_hbm)[which].at[b, g, rows], kv_buf.at[(g * 2 + which) * NB + b, rows],
              sem_a.at[g], priority)

    def fetch_b(s, which, i, r):
        slot = s % NSLOT
        rows = _rows(r, CH)
        sem = sem_v.at[2 * slot + int(r * CH >= V_SPLIT)] if which else sem_k.at[slot]
        fetch((kb_hbm, vb_hbm)[which].at[2 * i + s % 2, s // 2, rows],
              kv_buf.at[B_BASE + (slot * 2 + which) * HB + i, rows], sem, which)

    def fetch_half_step(u, half):
        def issue(with_a):
            for r in range(half * NCH // 2, (half + 1) * NCH // 2):
                for i in range(HB):
                    fetch_b(u, 0, i, r)
                    fetch_b(u, 1, HB - 1 - i, r)
                if with_a:
                    fetch_a(u + A_AHEAD, 0, r, 0)
                    fetch_a(u + A_AHEAD, 1, r, 1)

        pl.when(u < NSTEP - A_AHEAD)(lambda: issue(True))
        pl.when(jnp.logical_and(u >= NSTEP - A_AHEAD, u < NSTEP))(lambda: issue(False))

    for c in range(NB * SQ // WO_ROWS):
        rows = _rows(c, WO_ROWS)
        fetch(xa_hbm.at[rows], x_buf.at[0, rows], sem_x, 1)
        fetch(xb_hbm.at[rows], x_buf.at[1, rows], sem_x, 1)

    @pl.loop(0, W_CHUNKS // W_STREAMS)
    def _(i):
        for n in range(W_STREAMS):
            c = n * (W_CHUNKS // W_STREAMS) + i
            rows, cols = _rows(c // 2, WQ_ROWS), _rows(c % 2, WQ_COLS)
            fetch(wqa_hbm.at[rows, cols], wq_buf.at[0, rows, cols], sem_wq, 0)
            fetch(wqb_hbm.at[rows, cols], wq_buf.at[1, rows, cols], sem_wq, 1)

    @pl.loop(0, W_CHUNKS // W_STREAMS)
    def _(i):
        for n in range(W_STREAMS):
            rows = _rows(n * (W_CHUNKS // W_STREAMS) + i, WO_ROWS)
            fetch(woa_hbm.at[rows], wo_buf.at[0, rows], sem_wo, 0)
            fetch(wob_hbm.at[rows], wo_buf.at[1, rows], sem_wo, 1)

    @pl.loop(0, A_AHEAD)
    def _(a):
        for which in range(2):
            for b in range(HB):
                fetch_a(a, which, b, 0)
                fetch_a(a, which, b + HB, 1)

    @pl.loop(0, NB)
    def _(b):
        acc[0, _rows(b, SQ), :] = jnp.zeros((SQ, D), F32)
        acc[1, _rows(b, SQ), :] = jnp.zeros((SQ, D), F32)

    wait_filled(x_buf, sem_x)
    wait_filled(wq_buf, sem_wq)
    wait_filled(wo_buf, sem_wo)

    def store_out(rows, cols):
        pltpu.make_async_copy(out_buf.at[rows, cols], out_hbm.at[rows, cols], sem_out).start()

    def gqa_unit(u):
        g, b = u // NB, u % NB

        @pl.when(b == 0)
        def _():
            wait_filled(kv_buf.at[pl.ds(g * 2 * NB, 2 * NB)], sem_a.at[g])

        rows, group = _rows(b, SQ), _rows(g, GW)
        q = jnp.dot(x_buf[0, rows, :], wq_buf[0, :, group], preferred_element_type=F32)
        q = (q * Q_SCALE).astype(BF16)
        pairs = [jnp.concatenate([q[:, j * DH:(j + 1) * DH], q[:, (j + 1) * DH:(j + 2) * DH]], axis=0)
                 for j in range(0, REP, 2)]
        scores = [_softmax_scores(qp, kv_buf[g * 2 * NB + b]) for qp in pairs]
        o = [_weighted_values(sc, kv_buf[(g * 2 + 1) * NB + b]) for sc in scores]
        o = jnp.concatenate([op[j * SQ:(j + 1) * SQ] for op in o for j in range(2)], axis=1)
        total = acc[0, rows, :] + jnp.dot(o, wo_buf[0, group, :], preferred_element_type=F32)
        acc[0, rows, :] = total
        out_buf[rows, 0:D] = total.astype(BF16)

    def mha_step(t):
        slot, parity, head = t % NSLOT, t % 2, _rows(t // 2, DH)
        k0 = B_BASE + slot * 2 * HB
        v0 = k0 + HB
        batch_rows = [_rows(2 * i + parity, SQ) for i in range(HB)]

        wait_filled(kv_buf.at[pl.ds(k0, HB)], sem_k.at[slot])
        x = jnp.concatenate([x_buf[1, rows, :] for rows in batch_rows], axis=0)
        q = jnp.dot(x, wq_buf[1, :, head], preferred_element_type=F32)
        q = (q * Q_SCALE).astype(BF16)
        scores = [_softmax_scores(q[i * SQ:(i + 1) * SQ], kv_buf[k0 + i]) for i in range(HB)]

        wait_filled(kv_buf.at[pl.ds(v0, HB), pl.ds(0, V_SPLIT)], sem_v.at[2 * slot])

        @pl.when(t == NSTEP - 1)
        def _():
            store_out(slice(None), pl.ds(0, D))
            for i in range(HB):
                store_out(_rows(2 * i, SQ), pl.ds(D, D))

        wait_filled(kv_buf.at[pl.ds(v0, HB), pl.ds(V_SPLIT, SK - V_SPLIT)], sem_v.at[2 * slot + 1])

        o = jnp.concatenate([_weighted_values(scores[i], kv_buf[v0 + i]) for i in range(HB)], axis=0)
        acc_rows = _rows(parity, HB * SQ)
        total = jnp.dot(o, wo_buf[1, head, :], preferred_element_type=F32) + acc[1, acc_rows, :]
        acc[1, acc_rows, :] = total
        for i in range(HB):
            out_buf[batch_rows[i], D:2 * D] = total[i * SQ:(i + 1) * SQ].astype(BF16)

    @pl.loop(0, NSTEP + LAG)
    def _(u):
        fetch_half_step(u, 0)
        pl.when(u < NSTEP)(lambda: gqa_unit(u))
        fetch_half_step(u, 1)
        pl.when(u >= LAG)(lambda: mha_step(u - LAG))

    for i in range(HB):
        store_out(_rows(2 * i + 1, SQ), pl.ds(D, D))
    pltpu.make_async_copy(out_buf, out_hbm, sem_out).wait()


@jax.jit
def pallas_concat_heads__gqa_block_cached__mha_block_cached__near_ridge_kernel(
    A_x: jax.Array,
    A_k_cache: jax.Array,
    A_v_cache: jax.Array,
    A_wq: jax.Array,
    A_wo: jax.Array,
    B_x: jax.Array,
    B_k_cache: jax.Array,
    B_v_cache: jax.Array,
    B_wq: jax.Array,
    B_wo: jax.Array,
):
    assert A_x.shape == B_x.shape == (NB, SQ, D)
    assert A_k_cache.shape == A_v_cache.shape == (NB, HKV, SK, DH)
    assert B_k_cache.shape == B_v_cache.shape == (NB, HQ, SK, DH)
    assert A_wq.shape == B_wq.shape == (D, HQ * DH)
    assert A_wo.shape == B_wo.shape == (HQ * DH, D)

    hbm = pl.BlockSpec(memory_space=pltpu.HBM)
    out = pl.pallas_call(
        _kernel,
        out_shape=jax.ShapeDtypeStruct((NB * SQ, 2 * D), BF16),
        in_specs=[hbm] * 10,
        out_specs=hbm,
        scratch_shapes=[
            pltpu.VMEM((2, NB * SQ, D), BF16),
            pltpu.VMEM((2, D, HQ * DH), BF16),
            pltpu.VMEM((2, HQ * DH, D), BF16),
            pltpu.VMEM((B_BASE + NSLOT * 2 * HB, SK, DH), BF16),
            pltpu.VMEM((2, NB * SQ, D), F32),
            pltpu.VMEM((NB * SQ, 2 * D), BF16),
            pltpu.SemaphoreType.DMA,
            pltpu.SemaphoreType.DMA,
            pltpu.SemaphoreType.DMA,
            pltpu.SemaphoreType.DMA((HKV,)),
            pltpu.SemaphoreType.DMA((NSLOT,)),
            pltpu.SemaphoreType.DMA((2 * NSLOT,)),
            pltpu.SemaphoreType.DMA,
        ],
        compiler_params=pltpu.CompilerParams(
            vmem_limit_bytes=100 * 1024 * 1024,
            disable_bounds_checks=True,
            disable_semaphore_checks=True,
        ),
    )(A_x.reshape(NB * SQ, D), A_k_cache, A_v_cache, A_wq, A_wo,
      B_x.reshape(NB * SQ, D), B_k_cache, B_v_cache, B_wq, B_wo)
    return out.reshape(NB, SQ, 2 * D)
```

```python
import math

import jax
import jax.numpy as jnp
from jax import lax
import jax.experimental.pallas as pl
import jax.experimental.pallas.tpu as pltpu

NB, SQ, D = 8, 48, 512
HQ, HKV, SK, DH = 32, 8, 1024, 128
REP = HQ // HKV
GW = REP * DH
NSTEP = HKV * NB
HB = NB // 2

CH = 128
NCH = SK // CH
WO_ROWS = 32
WQ_ROWS, WQ_COLS = 8, 2048
W_CHUNKS = HQ * DH // WO_ROWS
W_STREAMS = 4

LAG = 2
NSLOT = 4
A_AHEAD = 2 * NCH
V_SPLIT = 6 * CH
B_BASE = HKV * 2 * NB

Q_SCALE = DH ** -0.5 * math.log2(math.e)

BF16, F32 = jnp.bfloat16, jnp.float32


def _rows(index, size):
    if isinstance(index, int):
        return pl.ds(index * size, size)
    return pl.ds(pl.multiple_of(index * size, size), size)


def _softmax_scores(q, k):
    s = lax.dot_general(q, k, (((1,), (1,)), ((), ())), preferred_element_type=F32)
    p = jnp.exp2(s - jnp.max(s, axis=-1, keepdims=True))
    return p.astype(BF16), 1.0 / jnp.sum(p, axis=-1, keepdims=True)


def _weighted_values(scores, v):
    p, inv_sum = scores
    return (jnp.dot(p, v, preferred_element_type=F32) * inv_sum).astype(BF16)


def _kernel(xa_hbm, ka_hbm, va_hbm, wqa_hbm, woa_hbm,
            xb_hbm, kb_hbm, vb_hbm, wqb_hbm, wob_hbm, out_hbm,
            x_buf, wq_buf, wo_buf, kv_buf, acc, out_a, out_b,
            sem_x, sem_wq, sem_wo, sem_a, sem_k, sem_v, sem_out):

    def fetch(src, dst, sem, priority):
        pltpu.make_async_copy(src, dst, sem).start(priority=priority)

    def wait_filled(buf, sem):
        pltpu.make_async_copy(buf, buf, sem).wait()

    def fetch_a(a, which, b, priority):
        g = a // NCH
        rows = _rows(a % NCH, CH)
        fetch((ka_hbm, va_hbm)[which].at[b, g, rows], kv_buf.at[(g * 2 + which) * NB + b, rows],
              sem_a.at[g], priority)

    def fetch_b(s, which, i, r):
        slot = s % NSLOT
        rows = _rows(r, CH)
        sem = sem_v.at[2 * slot + int(r * CH >= V_SPLIT)] if which else sem_k.at[slot]
        fetch((kb_hbm, vb_hbm)[which].at[2 * i + s % 2, s // 2, rows],
              kv_buf.at[B_BASE + (slot * 2 + which) * HB + i, rows], sem, which)

    def fetch_half_step(u, half):
        def issue(with_a):
            for r in range(half * NCH // 2, (half + 1) * NCH // 2):
                for i in range(HB):
                    fetch_b(u, 0, i, r)
                    fetch_b(u, 1, HB - 1 - i, r)
                if with_a:
                    fetch_a(u + A_AHEAD, 0, r, 0)
                    fetch_a(u + A_AHEAD, 1, r, 1)

        pl.when(u < NSTEP - A_AHEAD)(lambda: issue(True))
        pl.when(jnp.logical_and(u >= NSTEP - A_AHEAD, u < NSTEP))(lambda: issue(False))

    for c in range(NB * SQ // WO_ROWS):
        rows = _rows(c, WO_ROWS)
        fetch(xa_hbm.at[rows], x_buf.at[0, rows], sem_x, 1)
        fetch(xb_hbm.at[rows], x_buf.at[1, rows], sem_x, 1)

    @pl.loop(0, W_CHUNKS // W_STREAMS)
    def _(i):
        for n in range(W_STREAMS):
            c = n * (W_CHUNKS // W_STREAMS) + i
            rows, cols = _rows(c // 2, WQ_ROWS), _rows(c % 2, WQ_COLS)
            fetch(wqa_hbm.at[rows, cols], wq_buf.at[0, rows, cols], sem_wq, 0)
            fetch(wqb_hbm.at[rows, cols], wq_buf.at[1, rows, cols], sem_wq, 1)

    @pl.loop(0, W_CHUNKS // W_STREAMS)
    def _(i):
        for n in range(W_STREAMS):
            rows = _rows(n * (W_CHUNKS // W_STREAMS) + i, WO_ROWS)
            fetch(woa_hbm.at[rows], wo_buf.at[0, rows], sem_wo, 0)
            fetch(wob_hbm.at[rows], wo_buf.at[1, rows], sem_wo, 1)

    @pl.loop(0, A_AHEAD)
    def _(a):
        for which in range(2):
            for b in range(HB):
                fetch_a(a, which, b, 0)
                fetch_a(a, which, b + HB, 1)

    @pl.loop(0, NB)
    def _(b):
        acc[0, _rows(b, SQ), :] = jnp.zeros((SQ, D), F32)
        acc[1, _rows(b, SQ), :] = jnp.zeros((SQ, D), F32)

    wait_filled(x_buf, sem_x)
    wait_filled(wq_buf, sem_wq)
    wait_filled(wo_buf, sem_wo)

    def store_a():
        return pltpu.make_async_copy(out_a, out_hbm.at[:, pl.ds(0, D)], sem_out)

    def store_b(parity, i):
        return pltpu.make_async_copy(out_b.at[parity, _rows(i, SQ)],
                                     out_hbm.at[_rows(2 * i + parity, SQ), pl.ds(D, D)], sem_out)

    def gqa_unit(u):
        g, b = u // NB, u % NB

        @pl.when(b == 0)
        def _():
            wait_filled(kv_buf.at[pl.ds(g * 2 * NB, 2 * NB)], sem_a.at[g])

        rows, group = _rows(b, SQ), _rows(g, GW)
        q = jnp.dot(x_buf[0, rows, :], wq_buf[0, :, group], preferred_element_type=F32)
        q = (q * Q_SCALE).astype(BF16)
        pairs = [jnp.concatenate([q[:, j * DH:(j + 1) * DH], q[:, (j + 1) * DH:(j + 2) * DH]], axis=0)
                 for j in range(0, REP, 2)]
        scores = [_softmax_scores(qp, kv_buf[g * 2 * NB + b]) for qp in pairs]
        o = [_weighted_values(sc, kv_buf[(g * 2 + 1) * NB + b]) for sc in scores]
        o = jnp.concatenate([op[j * SQ:(j + 1) * SQ] for op in o for j in range(2)], axis=1)
        total = acc[0, rows, :] + jnp.dot(o, wo_buf[0, group, :], preferred_element_type=F32)
        acc[0, rows, :] = total
        out_a[rows, :] = total.astype(BF16)

    def mha_step(t):
        slot, parity, head = t % NSLOT, t % 2, _rows(t // 2, DH)
        k0 = B_BASE + slot * 2 * HB
        v0 = k0 + HB

        wait_filled(kv_buf.at[pl.ds(k0, HB)], sem_k.at[slot])
        x = jnp.concatenate([x_buf[1, _rows(2 * i + parity, SQ), :] for i in range(HB)], axis=0)
        q = jnp.dot(x, wq_buf[1, :, head], preferred_element_type=F32)
        q = (q * Q_SCALE).astype(BF16)
        scores = [_softmax_scores(q[i * SQ:(i + 1) * SQ], kv_buf[k0 + i]) for i in range(HB)]

        wait_filled(kv_buf.at[pl.ds(v0, HB), pl.ds(0, V_SPLIT)], sem_v.at[2 * slot])

        @pl.when(t == NSTEP - 1)
        def _():
            store_a().start()
            for i in range(HB):
                store_b(0, i).start()

        wait_filled(kv_buf.at[pl.ds(v0, HB), pl.ds(V_SPLIT, SK - V_SPLIT)], sem_v.at[2 * slot + 1])

        o = jnp.concatenate([_weighted_values(scores[i], kv_buf[v0 + i]) for i in range(HB)], axis=0)
        acc_rows = _rows(parity, HB * SQ)
        total = jnp.dot(o, wo_buf[1, head, :], preferred_element_type=F32) + acc[1, acc_rows, :]
        acc[1, acc_rows, :] = total
        out_b[parity] = total.astype(BF16)

    @pl.loop(0, NSTEP + LAG)
    def _(u):
        pl.when(u < NSTEP)(lambda: gqa_unit(u))
        fetch_half_step(u, 0)
        pl.when(u >= LAG)(lambda: mha_step(u - LAG))
        fetch_half_step(u, 1)

    for i in range(HB):
        store_b(1, i).start()
    store_a().wait()
    for parity in range(2):
        for i in range(HB):
            store_b(parity, i).wait()


@jax.jit
def pallas_concat_heads__gqa_block_cached__mha_block_cached__near_ridge_kernel(
    A_x: jax.Array,
    A_k_cache: jax.Array,
    A_v_cache: jax.Array,
    A_wq: jax.Array,
    A_wo: jax.Array,
    B_x: jax.Array,
    B_k_cache: jax.Array,
    B_v_cache: jax.Array,
    B_wq: jax.Array,
    B_wo: jax.Array,
):
    assert A_x.shape == B_x.shape == (NB, SQ, D)
    assert A_k_cache.shape == A_v_cache.shape == (NB, HKV, SK, DH)
    assert B_k_cache.shape == B_v_cache.shape == (NB, HQ, SK, DH)
    assert A_wq.shape == B_wq.shape == (D, HQ * DH)
    assert A_wo.shape == B_wo.shape == (HQ * DH, D)

    hbm = pl.BlockSpec(memory_space=pltpu.HBM)
    out = pl.pallas_call(
        _kernel,
        out_shape=jax.ShapeDtypeStruct((NB * SQ, 2 * D), BF16),
        in_specs=[hbm] * 10,
        out_specs=hbm,
        scratch_shapes=[
            pltpu.VMEM((2, NB * SQ, D), BF16),
            pltpu.VMEM((2, D, HQ * DH), BF16),
            pltpu.VMEM((2, HQ * DH, D), BF16),
            pltpu.VMEM((B_BASE + NSLOT * 2 * HB, SK, DH), BF16),
            pltpu.VMEM((2, NB * SQ, D), F32),
            pltpu.VMEM((NB * SQ, D), BF16),
            pltpu.VMEM((2, HB * SQ, D), BF16),
            pltpu.SemaphoreType.DMA,
            pltpu.SemaphoreType.DMA,
            pltpu.SemaphoreType.DMA,
            pltpu.SemaphoreType.DMA((HKV,)),
            pltpu.SemaphoreType.DMA((NSLOT,)),
            pltpu.SemaphoreType.DMA((2 * NSLOT,)),
            pltpu.SemaphoreType.DMA,
        ],
        compiler_params=pltpu.CompilerParams(
            vmem_limit_bytes=100 * 1024 * 1024,
            disable_bounds_checks=True,
            disable_semaphore_checks=True,
        ),
    )(A_x.reshape(NB * SQ, D), A_k_cache, A_v_cache, A_wq, A_wo,
      B_x.reshape(NB * SQ, D), B_k_cache, B_v_cache, B_wq, B_wo)
    return out.reshape(NB, SQ, 2 * D)
```
